```python
import os as _os
_os.environ.setdefault("JAX_PLATFORMS", "cpu")
import jax
import jax.numpy as jnp

def _softmax(x, axis=-1):
    return jax.nn.softmax(x, axis=axis)
def _gelu(x):
    return jax.nn.gelu(x, approximate=True)
def _silu(x):
    return jax.nn.silu(x)
def _sigmoid(x):
    return jax.nn.sigmoid(x)
def _layernorm(x, axis=-1, eps=1e-5):
    m = jnp.mean(x, axis=axis, keepdims=True)
    v = jnp.var(x, axis=axis, keepdims=True)
    return (x - m) / jnp.sqrt(v + eps)
def _scatter_add(tgt, idx, src, axis=0):
    return tgt.at[idx].add(src)
def _segment_sum(src, seg, n):
    return jax.ops.segment_sum(src, seg, n)
class _Rng:
    def __init__(self, key):
        self._k = key
    def _next(self):
        self._k, sub = jax.random.split(self._k)
        return sub
    def normal(self, shape):
        return jax.random.normal(self._next(), shape, dtype=jnp.bfloat16)
    def randint(self, lo, hi, shape):
        return jax.random.randint(self._next(), shape, lo, hi, dtype=jnp.int32)
    def uniform(self, shape, lo=0.0, hi=1.0):
        return jax.random.uniform(self._next(), shape, jnp.bfloat16, lo, hi)
    def permutation(self, n):
        return jax.random.permutation(self._next(), n)


kernel_name = 'gated_mix__gqa_block_cached__dense_activation_squared_relu__decode'

def setup_inputs():
    _rng = _Rng(jax.random.key(int.from_bytes(__import__("os").urandom(4), "little")))
    _w = (lambda a: (lambda t: t.astype(jnp.bfloat16) if jnp.issubdtype(t.dtype, jnp.floating) else t)(jnp.asarray(a)))
    def _A_setup():
        B, Sq, D = 4, 1, 512
        Hq, Hkv, Sk, Dh = 32, 8, 4096, 128
        assert Hq % Hkv == 0, (Hq, Hkv)
        return {
            "x": _w((lambda *s: _rng.normal(s) * 0.05)(B, Sq, D)),
            "k_cache": _w((lambda *s: _rng.normal(s) * 3.2)(B, Hkv, Sk, Dh)),
            "v_cache": _w((lambda *s: _rng.normal(s) * 1.6)(B, Hkv, Sk, Dh)),
            "wq": _w((lambda *s: _rng.normal(s) * 3.2)(D, Hq * Dh) * (D ** -0.5)),
            "wo": _w((lambda *s: _rng.normal(s) * 1.6)(Hq * Dh, D) * ((Hq * Dh) ** -0.5)),
        }
    _A_in = _A_setup()

    def _B_setup():
        B, S, D, F = 4, 1, 512, 1792
        return {
            "x": _w((lambda *s: _rng.normal(s) * 0.05)(B, S, D)),
            "w1": _w((lambda *s: _rng.normal(s) * 0.1)(D, F)),
            "b1": _w((lambda *s: _rng.normal(s) * 0.05)(F)),
            "w2": _w((lambda *s: _rng.normal(s) * 0.05)(F, D)),
            "b2": _w((lambda *s: _rng.normal(s) * 0.05)(D)),
        }
    _B_in = _B_setup()

    return {
        "A_x": _A_in["x"],
        "A_k_cache": _A_in["k_cache"],
        "A_v_cache": _A_in["v_cache"],
        "A_wq": _A_in["wq"],
        "A_wo": _A_in["wo"],
        "B_x": _B_in["x"],
        "B_w1": _B_in["w1"],
        "B_b1": _B_in["b1"],
        "B_w2": _B_in["w2"],
        "B_b2": _B_in["b2"],
        "gate_w": _w((lambda *s: _rng.normal(s) * 0.05)(512) * 16.0),
    }

def reference(A_x, A_k_cache, A_v_cache, A_wq, A_wo, B_x, B_w1, B_b1, B_w2, B_b2, gate_w):
    def _A_ref(x, k_cache, v_cache, wq, wo):
        B, Sq, D = x.shape
        Hq, Dh = 32, 128
        Hkv = k_cache.shape[1]
        rep = Hq // Hkv
        q = (lambda x, *d: x.transpose(*d))((x @ wq).reshape(B, Sq, Hq, Dh), 0, 2, 1, 3)
        k = jnp.repeat(k_cache, rep, axis=1)
        v = jnp.repeat(v_cache, rep, axis=1)
        scores = jnp.einsum("bhqd,bhkd->bhqk", q, k) * (Dh ** -0.5)
        p = _softmax(scores, axis=-1)
        o = jnp.einsum("bhqk,bhkd->bhqd", p, v)
        return (lambda x, *d: x.transpose(*d))(o, 0, 2, 1, 3).reshape(B, Sq, Hq * Dh) @ wo

    def _B_ref(x, w1, b1, w2, b2):
        h = jnp.einsum("bsd,df->bsf", x, w1) + b1
        zero = jnp.zeros_like(h)
        r = jnp.where(h > zero, h, zero)
        h = r * r
        out = jnp.einsum("bsf,fd->bsd", h, w2) + b2
        return out

    x = A_x
    g = _sigmoid((x * gate_w).sum(-1, keepdims=True))
    a = _A_ref(x, A_k_cache, A_v_cache, A_wq, A_wo)
    b = _B_ref(x, B_w1, B_b1, B_w2, B_b2)
    return g * a + (1 - g) * b
```

```python
import functools
import jax
import jax.numpy as jnp
from jax import lax
from jax.experimental import pallas as pl
from jax.experimental.pallas import tpu as pltpu

B, D, HQ, HKV, SK, DH, F = 4, 512, 32, 8, 4096, 128, 1792
REP = HQ // HKV
NP = B * HKV
F32, BF16 = jnp.float32, jnp.bfloat16

def make_kernel(w2_tiles=(8, 5, 1), wo_last=False):
    w2_chunks = []
    off = 0
    for t in w2_tiles:
        w2_chunks.append((off * 128, t * 128)); off += t
    assert off * 128 == F

    def kernel(x_hbm, k_hbm, v_hbm, wq_hbm, wo_hbm, w1_hbm, b1_hbm, w2_hbm, b2_hbm, gw_hbm,
               o_ref,
               xb, kb, vb, wqb, wob, w1b, b1b, w2b, b2b, gwb, q_scr, o_scr, sem):
        s0, s1 = sem.at[0], sem.at[1]
        def k_copy(p):
            return pltpu.make_async_copy(k_hbm.at[p // HKV, p % HKV], kb.at[p], s0)
        def v_copy(p):
            return pltpu.make_async_copy(v_hbm.at[p // HKV, p % HKV], vb.at[p], s1)
        a0 = [pltpu.make_async_copy(s, d, s0) for (s, d) in
              [(wq_hbm, wqb), (x_hbm, xb), (gw_hbm, gwb), (b1_hbm, b1b), (b2_hbm, b2b)]]
        a1 = pltpu.make_async_copy(w1_hbm, w1b, s1)
        wo_cp = pltpu.make_async_copy(wo_hbm, wob, s0)
        w2_cp = [pltpu.make_async_copy(w2_hbm.at[pl.ds(o, n)], w2b.at[pl.ds(o, n)], sem.at[(i + 1) % 2])
                 for i, (o, n) in enumerate(w2_chunks)]
        for c in a0: c.start()
        a1.start()
        for c in a0: c.wait()
        k_copy(0).start()
        x4 = xb[...]
        row = lax.broadcasted_iota(jnp.int32, (16, D), 0)
        xrep = jnp.concatenate([x4[b:b+1] for b in range(B) for _ in range(4)], axis=0).astype(F32)
        lhs = [jnp.where(row % 4 == r, xrep, 0.0).astype(BF16) for r in range(REP)]
        for h in range(HKV):
            acc = jnp.zeros((16, DH), F32)
            for r in range(REP):
                t = h * REP + r
                acc += jnp.dot(lhs[r], wqb[:, t * DH:(t + 1) * DH], preferred_element_type=F32)
            q_scr[h] = acc
        a1.wait()
        v_copy(0).start()
        x8 = jnp.concatenate([x4, x4], axis=0)
        hpre = jnp.dot(x8, w1b[...], preferred_element_type=F32) + b1b[...].astype(F32)[None, :]
        rl = jnp.where(hpre > 0, hpre, 0.0)
        r2 = (rl * rl).astype(BF16)
        gate = jax.nn.sigmoid(jnp.sum(x8.astype(F32) * gwb[...].astype(F32)[None, :], axis=-1, keepdims=True))

        scale = DH ** -0.5
        def body(p, carry):
            b = p // HKV; h = p % HKV
            k_copy(p).wait()
            @pl.when(p < NP - 1)
            def _():
                k_copy(p + 1).start()
            @pl.when(p == NP - 1)
            def _():
                wo_cp.start()
            j = b // 2
            sl = pl.ds(pl.multiple_of(j * 8, 8), 8)
            q8 = q_scr[h, sl, :].astype(BF16)
            s = lax.dot_general(q8, kb[p], (((1,), (1,)), ((), ())), preferred_element_type=F32) * scale
            m = jnp.max(s, axis=-1, keepdims=True)
            e = jnp.exp(s - m)
            l = jnp.sum(e, axis=-1, keepdims=True)
            v_copy(p).wait()
            @pl.when(p < NP - 1)
            def _():
                v_copy(p + 1).start()
            @pl.when(p == NP - 1)
            def _():
                w2_cp[0].start()
            o = jnp.dot(e.astype(BF16), vb[p], preferred_element_type=F32) / l
            rowi = lax.broadcasted_iota(jnp.int32, (8, DH), 0)
            keep = (rowi // 4) == (b % 2)
            @pl.when(b % 2 == 0)
            def _():
                o_scr[h, sl, :] = o
            @pl.when(b % 2 == 1)
            def _():
                o_scr[h, sl, :] = jnp.where(keep, o, o_scr[h, sl, :])
            return carry
        lax.fori_loop(0, NP, body, 0)

        rowo = lax.broadcasted_iota(jnp.int32, (16, DH), 0)
        los = []
        for t in range(HQ):
            h, r = t // REP, t % REP
            los.append(jnp.where(rowo % 4 == r, o_scr[h], 0.0).astype(BF16))
        lo = jnp.concatenate(los, axis=1)
        wo_cp.wait()
        if len(w2_cp) > 1: w2_cp[1].start()
        acc = jnp.dot(lo, wob[...], preferred_element_type=F32)
        a4 = jnp.concatenate([acc[4*b:4*b+1] + acc[4*b+1:4*b+2] + acc[4*b+2:4*b+3] + acc[4*b+3:4*b+4] for b in range(B)], axis=0)
        g4 = gate[0:4]
        gb = 1.0 - g4
        out = g4 * a4 + gb * b2b[...].astype(F32)[None, :]
        for i, (o_, n_) in enumerate(w2_chunks):
            w2_cp[i].wait()
            if i + 2 < len(w2_cp): w2_cp[i + 2].start()
            out = out + gb * jnp.dot(r2[:, o_:o_ + n_], w2b[o_:o_ + n_, :], preferred_element_type=F32)[0:4]
        o_ref[...] = out.astype(BF16)
    return kernel

def build(w2_tiles=(8, 5, 1), **cp):
    kernel = make_kernel(w2_tiles)
    def fn(A_x, A_k_cache, A_v_cache, A_wq, A_wo, B_x, B_w1, B_b1, B_w2, B_b2, gate_w):
        return pl.pallas_call(
            kernel,
            out_shape=jax.ShapeDtypeStruct((B, D), BF16),
            in_specs=[pl.BlockSpec(memory_space=pl.ANY)] * 10,
            out_specs=pl.BlockSpec(memory_space=pltpu.VMEM),
            scratch_shapes=[
                pltpu.VMEM((B, D), BF16), pltpu.VMEM((NP, SK, DH), BF16), pltpu.VMEM((NP, SK, DH), BF16),
                pltpu.VMEM((D, HQ * DH), BF16), pltpu.VMEM((HQ * DH, D), BF16), pltpu.VMEM((D, F), BF16),
                pltpu.VMEM((F,), BF16), pltpu.VMEM((F, D), BF16), pltpu.VMEM((D,), BF16), pltpu.VMEM((D,), BF16),
                pltpu.VMEM((HKV, 16, DH), F32), pltpu.VMEM((HKV, 16, DH), F32),
                pltpu.SemaphoreType.DMA((2,)),
            ],
            compiler_params=pltpu.CompilerParams(vmem_limit_bytes=110 * 1024 * 1024, **cp),
        )(A_x.reshape(B, D), A_k_cache, A_v_cache, A_wq, A_wo, B_w1, B_b1, B_w2, B_b2, gate_w).reshape(B, 1, D)
    return fn


_FN = build((8, 5, 1))


@jax.jit
def pallas_gated_mix__gqa_block_cached__dense_activation_squared_relu__decode_kernel(
    A_x: jax.Array,
    A_k_cache: jax.Array,
    A_v_cache: jax.Array,
    A_wq: jax.Array,
    A_wo: jax.Array,
    B_x: jax.Array,
    B_w1: jax.Array,
    B_b1: jax.Array,
    B_w2: jax.Array,
    B_b2: jax.Array,
    gate_w: jax.Array,
):
    return _FN(A_x, A_k_cache, A_v_cache, A_wq, A_wo, B_x, B_w1, B_b1, B_w2, B_b2, gate_w)
```

```python
import jax
import jax.numpy as jnp
from jax import lax
from jax.experimental import pallas as pl
from jax.experimental.pallas import tpu as pltpu

B, D, HQ, HKV, SK, DH, F = 4, 512, 32, 8, 4096, 128, 1792
REP = HQ // HKV
NP = B * HKV
F32, BF16 = jnp.float32, jnp.bfloat16
W2_ROWS = (1280, 384, 128)


def _kernel(x_hbm, k_hbm, v_hbm, wq_hbm, wo_hbm, w1_hbm, b1_hbm, w2_hbm, b2_hbm, gw_hbm,
            o_ref,
            xb, kb, vb, wqb, wob, w1b, b1b, w2b, b2b, gwb, q_scr, o_scr):
    w2_chunks, off = [], 0
    for n in W2_ROWS:
        w2_chunks.append((off, n))
        off += n

    def stream_and_compute(s0, s1):
        def k_copy(p):
            return pltpu.make_async_copy(k_hbm.at[p // HKV, p % HKV], kb.at[p], s0)

        def v_copy(p):
            return pltpu.make_async_copy(v_hbm.at[p // HKV, p % HKV], vb.at[p], s1)

        head_cps = [pltpu.make_async_copy(s, d, s0) for (s, d) in
                    [(wq_hbm, wqb), (x_hbm, xb), (gw_hbm, gwb), (b1_hbm, b1b), (b2_hbm, b2b)]]
        w1_cp = pltpu.make_async_copy(w1_hbm, w1b, s1)
        wo_cp = pltpu.make_async_copy(wo_hbm, wob, s0)
        w2_cps = [pltpu.make_async_copy(w2_hbm.at[pl.ds(o, n)], w2b.at[pl.ds(o, n)], sem)
                  for (o, n), sem in zip(w2_chunks, (s1, s0, s1))]

        for c in head_cps:
            c.start()
        w1_cp.start()
        for c in head_cps:
            c.wait()
        k_copy(0).start()

        x4 = xb[...]
        row = lax.broadcasted_iota(jnp.int32, (16, D), 0)
        xrep = jnp.concatenate([x4[b:b + 1] for b in range(B) for _ in range(REP)], axis=0).astype(F32)
        lhs = [jnp.where(row % REP == r, xrep, 0.0).astype(BF16) for r in range(REP)]
        for h in range(HKV):
            acc = jnp.zeros((16, DH), F32)
            for r in range(REP):
                t = h * REP + r
                acc += jnp.dot(lhs[r], wqb[:, t * DH:(t + 1) * DH], preferred_element_type=F32)
            q_scr[h] = acc

        w1_cp.wait()
        v_copy(0).start()
        x8 = jnp.concatenate([x4, x4], axis=0)
        hid = jnp.dot(x8, w1b[...], preferred_element_type=F32) + b1b[...].astype(F32)[None, :]
        hid = jnp.where(hid > 0, hid, 0.0)
        r2 = (hid * hid).astype(BF16)
        gate = jax.nn.sigmoid(
            jnp.sum(x8.astype(F32) * gwb[...].astype(F32)[None, :], axis=-1, keepdims=True))

        scale = DH ** -0.5

        def body(p, carry):
            b = p // HKV
            h = p % HKV
            k_copy(p).wait()

            @pl.when(p < NP - 1)
            def _():
                k_copy(p + 1).start()

            @pl.when(p == NP - 1)
            def _():
                wo_cp.start()

            sl = pl.ds(pl.multiple_of((b // 2) * 8, 8), 8)
            q8 = q_scr[h, sl, :].astype(BF16)
            s = lax.dot_general(q8, kb[p], (((1,), (1,)), ((), ())), preferred_element_type=F32) * scale
            m = jnp.max(s, axis=-1, keepdims=True)
            e = jnp.exp(s - m)
            l = jnp.sum(e, axis=-1, keepdims=True)

            v_copy(p).wait()

            @pl.when(p < NP - 1)
            def _():
                v_copy(p + 1).start()

            @pl.when(p == NP - 1)
            def _():
                w2_cps[0].start()

            o = jnp.dot(e.astype(BF16), vb[p], preferred_element_type=F32) / l
            keep = (lax.broadcasted_iota(jnp.int32, (8, DH), 0) // REP) == (b % 2)

            @pl.when(b % 2 == 0)
            def _():
                o_scr[h, sl, :] = o

            @pl.when(b % 2 == 1)
            def _():
                o_scr[h, sl, :] = jnp.where(keep, o, o_scr[h, sl, :])

            return carry

        lax.fori_loop(0, NP, body, 0)

        rowo = lax.broadcasted_iota(jnp.int32, (16, DH), 0)
        lo = jnp.concatenate(
            [jnp.where(rowo % REP == t % REP, o_scr[t // REP], 0.0).astype(BF16) for t in range(HQ)],
            axis=1)
        wo_cp.wait()
        w2_cps[1].start()
        acc = jnp.dot(lo, wob[...], preferred_element_type=F32)
        a4 = jnp.concatenate(
            [acc[4 * b:4 * b + 1] + acc[4 * b + 1:4 * b + 2] + acc[4 * b + 2:4 * b + 3] + acc[4 * b + 3:4 * b + 4]
             for b in range(B)], axis=0)
        g4 = gate[0:4]
        gb = 1.0 - g4
        out = g4 * a4 + gb * b2b[...].astype(F32)[None, :]

        lhs2 = [r2[:, o_:o_ + n_] for (o_, n_) in w2_chunks]

        def w2_part(i):
            o_, n_ = w2_chunks[i]
            return jnp.dot(lhs2[i], w2b[o_:o_ + n_, :], preferred_element_type=F32)[0:4]

        w2_cps[0].wait()
        w2_cps[2].start()
        out = out + gb * w2_part(0)
        w2_cps[1].wait()
        out = out + gb * w2_part(1)
        w2_cps[2].wait()
        return out, gb, w2_part(2)

    out, gb, last = pl.run_scoped(
        stream_and_compute, pltpu.SemaphoreType.DMA(()), pltpu.SemaphoreType.DMA(()))
    o_ref[...] = (out + gb * last).astype(BF16)


@jax.jit
def pallas_gated_mix__gqa_block_cached__dense_activation_squared_relu__decode_kernel(
    A_x: jax.Array,
    A_k_cache: jax.Array,
    A_v_cache: jax.Array,
    A_wq: jax.Array,
    A_wo: jax.Array,
    B_x: jax.Array,
    B_w1: jax.Array,
    B_b1: jax.Array,
    B_w2: jax.Array,
    B_b2: jax.Array,
    gate_w: jax.Array,
):
    del B_x
    out = pl.pallas_call(
        _kernel,
        out_shape=jax.ShapeDtypeStruct((B, D), BF16),
        in_specs=[pl.BlockSpec(memory_space=pl.ANY)] * 10,
        out_specs=pl.BlockSpec(memory_space=pltpu.VMEM),
        scratch_shapes=[
            pltpu.VMEM((B, D), BF16),
            pltpu.VMEM((NP, SK, DH), BF16),
            pltpu.VMEM((NP, SK, DH), BF16),
            pltpu.VMEM((D, HQ * DH), BF16),
            pltpu.VMEM((HQ * DH, D), BF16),
            pltpu.VMEM((D, F), BF16),
            pltpu.VMEM((F,), BF16),
            pltpu.VMEM((F, D), BF16),
            pltpu.VMEM((D,), BF16),
            pltpu.VMEM((D,), BF16),
            pltpu.VMEM((HKV, 16, DH), F32),
            pltpu.VMEM((HKV, 16, DH), F32),
        ],
        compiler_params=pltpu.CompilerParams(vmem_limit_bytes=110 * 1024 * 1024),
    )(A_x.reshape(B, D), A_k_cache, A_v_cache, A_wq, A_wo, B_w1, B_b1, B_w2, B_b2, gate_w)
    return out.reshape(B, 1, D)
```

```python
import jax
import jax.numpy as jnp
from jax import lax
from jax.experimental import pallas as pl
from jax.experimental.pallas import tpu as pltpu

B, D, HQ, HKV, SK, DH, F = 4, 512, 32, 8, 4096, 128, 1792
REP = HQ // HKV
NP = B * HKV
F32, BF16 = jnp.float32, jnp.bfloat16
W2_ROWS = (1280, 384, 128)


def _kernel(x_hbm, k_hbm, v_hbm, wq_hbm, wo_hbm, w1_hbm, b1_hbm, w2_hbm, b2_hbm, gw_hbm,
            o_ref,
            xb, kb, vb, wqb, wob, w1b, b1b, w2b, b2b, gwb, q_scr, o_scr):
    w2_chunks, off = [], 0
    for n in W2_ROWS:
        w2_chunks.append((off, n))
        off += n

    def stream_and_compute(s0, s1):
        def k_copy(p):
            return pltpu.make_async_copy(k_hbm.at[p // HKV, p % HKV], kb.at[p], s0)

        def v_copy(p):
            return pltpu.make_async_copy(v_hbm.at[p // HKV, p % HKV], vb.at[p], s1)

        head_cps = [pltpu.make_async_copy(s, d, s0) for (s, d) in
                    [(wq_hbm, wqb), (x_hbm, xb), (gw_hbm, gwb), (b1_hbm, b1b), (b2_hbm, b2b)]]
        w1_cp = pltpu.make_async_copy(w1_hbm, w1b, s1)
        wo_cp = pltpu.make_async_copy(wo_hbm, wob, s0)
        w2_cps = [pltpu.make_async_copy(w2_hbm.at[pl.ds(o, n)], w2b.at[pl.ds(o, n)], sem)
                  for (o, n), sem in zip(w2_chunks, (s1, s0, s1))]

        for c in head_cps:
            c.start()
        w1_cp.start()
        for c in head_cps:
            c.wait()
        k_copy(0).start()

        x4 = xb[...]
        row = lax.broadcasted_iota(jnp.int32, (16, D), 0)
        xrep = jnp.concatenate([x4[b:b + 1] for b in range(B) for _ in range(REP)], axis=0).astype(F32)
        lhs = [jnp.where(row % REP == r, xrep, 0.0).astype(BF16) for r in range(REP)]
        for h in range(HKV):
            acc = jnp.zeros((16, DH), F32)
            for r in range(REP):
                t = h * REP + r
                acc += jnp.dot(lhs[r], wqb[:, t * DH:(t + 1) * DH], preferred_element_type=F32)
            q_scr[h] = acc

        w1_cp.wait()
        v_copy(0).start()
        x8 = jnp.concatenate([x4, x4], axis=0)
        hid = jnp.dot(x8, w1b[...], preferred_element_type=F32) + b1b[...].astype(F32)[None, :]
        hid = jnp.where(hid > 0, hid, 0.0)
        gate = jax.nn.sigmoid(
            jnp.sum(x8.astype(F32) * gwb[...].astype(F32)[None, :], axis=-1, keepdims=True))
        r2 = ((1.0 - gate) * (hid * hid)).astype(BF16)

        scale = DH ** -0.5

        def body(p, carry):
            b = p // HKV
            h = p % HKV
            k_copy(p).wait()

            @pl.when(p < NP - 1)
            def _():
                k_copy(p + 1).start()

            @pl.when(p == NP - 1)
            def _():
                wo_cp.start()

            sl = pl.ds(pl.multiple_of((b // 2) * 8, 8), 8)
            q8 = q_scr[h, sl, :].astype(BF16)
            s = lax.dot_general(q8, kb[p], (((1,), (1,)), ((), ())), preferred_element_type=F32) * scale
            m = jnp.max(s, axis=-1, keepdims=True)
            e = jnp.exp(s - m)
            l = jnp.sum(e, axis=-1, keepdims=True)

            v_copy(p).wait()

            @pl.when(p < NP - 1)
            def _():
                v_copy(p + 1).start()

            @pl.when(p == NP - 1)
            def _():
                w2_cps[0].start()

            o = jnp.dot(e.astype(BF16), vb[p], preferred_element_type=F32) / l
            keep = (lax.broadcasted_iota(jnp.int32, (8, DH), 0) // REP) == (b % 2)

            @pl.when(b % 2 == 0)
            def _():
                o_scr[h, sl, :] = o

            @pl.when(b % 2 == 1)
            def _():
                o_scr[h, sl, :] = jnp.where(keep, o, o_scr[h, sl, :])

            return carry

        lax.fori_loop(0, NP, body, 0)

        rowo = lax.broadcasted_iota(jnp.int32, (16, DH), 0)
        lo = jnp.concatenate(
            [jnp.where(rowo % REP == t % REP, o_scr[t // REP], 0.0).astype(BF16) for t in range(HQ)],
            axis=1)
        wo_cp.wait()
        w2_cps[1].start()
        acc = jnp.dot(lo, wob[...], preferred_element_type=F32)
        a4 = jnp.concatenate(
            [acc[4 * b:4 * b + 1] + acc[4 * b + 1:4 * b + 2] + acc[4 * b + 2:4 * b + 3] + acc[4 * b + 3:4 * b + 4]
             for b in range(B)], axis=0)
        def to16(v4):
            return jnp.concatenate([v4[:, j * 128:(j + 1) * 128] for j in range(D // 128)], axis=0)
        g16 = jnp.concatenate([gate[0:4]] * (D // 128), axis=0)
        b2r = b2b[...].astype(F32)[None, :]
        b2_16 = to16(jnp.broadcast_to(b2r, (4, D)))
        out = g16 * to16(a4) + (1.0 - g16) * b2_16

        lhs2 = [r2[:, o_:o_ + n_] for (o_, n_) in w2_chunks]
        low = lax.broadcasted_iota(jnp.int32, (8, 128), 0) < 4

        def w2_part(i):
            o_, n_ = w2_chunks[i]
            d = jnp.dot(lhs2[i], w2b[o_:o_ + n_, :], preferred_element_type=F32)
            return jnp.concatenate(
                [jnp.where(low, d[:, (2 * u) * 128:(2 * u + 1) * 128], d[:, (2 * u + 1) * 128:(2 * u + 2) * 128])
                 for u in range(2)], axis=0)

        w2_cps[0].wait()
        w2_cps[2].start()
        out = out + w2_part(0)
        w2_cps[1].wait()
        out = out + w2_part(1)
        w2_cps[2].wait()
        return out, w2_part(2)

    out, last = pl.run_scoped(
        stream_and_compute, pltpu.SemaphoreType.DMA(()), pltpu.SemaphoreType.DMA(()))
    o_ref[...] = (out + last).astype(BF16)


@jax.jit
def pallas_gated_mix__gqa_block_cached__dense_activation_squared_relu__decode_kernel(
    A_x: jax.Array,
    A_k_cache: jax.Array,
    A_v_cache: jax.Array,
    A_wq: jax.Array,
    A_wo: jax.Array,
    B_x: jax.Array,
    B_w1: jax.Array,
    B_b1: jax.Array,
    B_w2: jax.Array,
    B_b2: jax.Array,
    gate_w: jax.Array,
):
    del B_x
    out = pl.pallas_call(
        _kernel,
        out_shape=jax.ShapeDtypeStruct((16, 128), BF16),
        in_specs=[pl.BlockSpec(memory_space=pl.ANY)] * 10,
        out_specs=pl.BlockSpec(memory_space=pltpu.VMEM),
        scratch_shapes=[
            pltpu.VMEM((B, D), BF16),
            pltpu.VMEM((NP, SK, DH), BF16),
            pltpu.VMEM((NP, SK, DH), BF16),
            pltpu.VMEM((D, HQ * DH), BF16),
            pltpu.VMEM((HQ * DH, D), BF16),
            pltpu.VMEM((D, F), BF16),
            pltpu.VMEM((F,), BF16),
            pltpu.VMEM((F, D), BF16),
            pltpu.VMEM((D,), BF16),
            pltpu.VMEM((D,), BF16),
            pltpu.VMEM((HKV, 16, DH), F32),
            pltpu.VMEM((HKV, 16, DH), F32),
        ],
        compiler_params=pltpu.CompilerParams(vmem_limit_bytes=110 * 1024 * 1024),
    )(A_x.reshape(B, D), A_k_cache, A_v_cache, A_wq, A_wo, B_w1, B_b1, B_w2, B_b2, gate_w)
    return out.reshape(D // 128, B, 128).transpose(1, 0, 2).reshape(B, 1, D)
```

```python
import jax
import jax.numpy as jnp
from jax import lax
from jax.experimental import pallas as pl
from jax.experimental.pallas import tpu as pltpu

B, D, HQ, HKV, SK, DH, F = 4, 512, 32, 8, 4096, 128, 1792
REP = HQ // HKV
NP = B * HKV
F32, BF16 = jnp.float32, jnp.bfloat16
W2_ROWS = (1024, 384, 128)
W2V_ROWS = (64, 64, 64, 32, 24, 8)
NV = sum(W2V_ROWS)


def _kernel(x_hbm, k_hbm, v_hbm, wq_hbm, wo_hbm, w1_hbm, b1_hbm, w2_hbm, b2_hbm, gw_hbm,
            o_ref,
            xb, kb, vb, wqb, wob, w1b, b1b, w2b, b2b, gwb, q_scr, o_scr, p_scr):
    w2_chunks, off = [], 0
    for n in W2_ROWS + W2V_ROWS:
        w2_chunks.append((off, n))
        off += n
    assert off == F
    NM = len(W2_ROWS)

    def stream_and_compute(s0, s1, *sw):
        def k_copy(p):
            return pltpu.make_async_copy(k_hbm.at[p // HKV, p % HKV], kb.at[p], s0)

        def v_copy(p):
            return pltpu.make_async_copy(v_hbm.at[p // HKV, p % HKV], vb.at[p], s1)

        head_cps = [pltpu.make_async_copy(s, d, s0) for (s, d) in
                    [(wq_hbm, wqb), (x_hbm, xb), (gw_hbm, gwb), (b1_hbm, b1b), (b2_hbm, b2b)]]
        w1_cp = pltpu.make_async_copy(w1_hbm, w1b, s1)
        wo_cp = pltpu.make_async_copy(wo_hbm, wob, s0)
        w2_cps = [pltpu.make_async_copy(w2_hbm.at[pl.ds(o, n)], w2b.at[pl.ds(o, n)], sem)
                  for (o, n), sem in zip(w2_chunks, sw)]

        for c in head_cps:
            c.start()
        w1_cp.start()
        for c in head_cps:
            c.wait()
        k_copy(0).start()

        x4 = xb[...]
        row = lax.broadcasted_iota(jnp.int32, (16, D), 0)
        xrep = jnp.concatenate([x4[b:b + 1] for b in range(B) for _ in range(REP)], axis=0).astype(F32)
        lhs = [jnp.where(row % REP == r, xrep, 0.0).astype(BF16) for r in range(REP)]
        for h in range(HKV):
            acc = jnp.zeros((16, DH), F32)
            for r in range(REP):
                t = h * REP + r
                acc += jnp.dot(lhs[r], wqb[:, t * DH:(t + 1) * DH], preferred_element_type=F32)
            q_scr[h] = acc

        w1_cp.wait()
        v_copy(0).start()
        x8 = jnp.concatenate([x4, x4], axis=0)
        hid = jnp.dot(x8, w1b[...], preferred_element_type=F32) + b1b[...].astype(F32)[None, :]
        hid = jnp.where(hid > 0, hid, 0.0)
        gate = jax.nn.sigmoid(
            jnp.sum(x8.astype(F32) * gwb[...].astype(F32)[None, :], axis=-1, keepdims=True))
        r2f = (1.0 - gate) * (hid * hid)
        r2 = r2f.astype(BF16)
        for t in range(NV // 128):
            rt = r2f[:, F - NV + t * 128:F - NV + (t + 1) * 128].T
            for b in range(B):
                p_scr[b, t * 128:(t + 1) * 128, :] = jnp.broadcast_to(rt[:, b:b + 1], (128, 128))

        scale = DH ** -0.5

        def body(p, carry):
            b = p // HKV
            h = p % HKV
            k_copy(p).wait()

            @pl.when(p < NP - 1)
            def _():
                k_copy(p + 1).start()

            @pl.when(p == NP - 1)
            def _():
                wo_cp.start()

            sl = pl.ds(pl.multiple_of((b // 2) * 8, 8), 8)
            q8 = q_scr[h, sl, :].astype(BF16)
            s = lax.dot_general(q8, kb[p], (((1,), (1,)), ((), ())), preferred_element_type=F32) * scale
            m = jnp.max(s, axis=-1, keepdims=True)
            e = jnp.exp(s - m)
            l = jnp.sum(e, axis=-1, keepdims=True)

            v_copy(p).wait()

            @pl.when(p < NP - 1)
            def _():
                v_copy(p + 1).start()

            @pl.when(p == NP - 1)
            def _():
                for c in w2_cps:
                    c.start()

            o = jnp.dot(e.astype(BF16), vb[p], preferred_element_type=F32) / l
            keep = (lax.broadcasted_iota(jnp.int32, (8, DH), 0) // REP) == (b % 2)

            @pl.when(b % 2 == 0)
            def _():
                o_scr[h, sl, :] = o

            @pl.when(b % 2 == 1)
            def _():
                o_scr[h, sl, :] = jnp.where(keep, o, o_scr[h, sl, :])

            return carry

        lax.fori_loop(0, NP, body, 0)

        rowo = lax.broadcasted_iota(jnp.int32, (16, DH), 0)
        lo = jnp.concatenate(
            [jnp.where(rowo % REP == t % REP, o_scr[t // REP], 0.0).astype(BF16) for t in range(HQ)],
            axis=1)
        wo_cp.wait()
        acc = jnp.dot(lo, wob[...], preferred_element_type=F32)
        a4 = jnp.concatenate(
            [acc[4 * b:4 * b + 1] + acc[4 * b + 1:4 * b + 2] + acc[4 * b + 2:4 * b + 3] + acc[4 * b + 3:4 * b + 4]
             for b in range(B)], axis=0)
        def to16(v4):
            return jnp.concatenate([v4[:, j * 128:(j + 1) * 128] for j in range(D // 128)], axis=0)
        g16 = jnp.concatenate([gate[0:4]] * (D // 128), axis=0)
        b2r = b2b[...].astype(F32)[None, :]
        b2_16 = to16(jnp.broadcast_to(b2r, (4, D)))
        out = g16 * to16(a4) + (1.0 - g16) * b2_16

        lhs2 = [r2[:, o_:o_ + n_] for (o_, n_) in w2_chunks[:NM]]
        low = lax.broadcasted_iota(jnp.int32, (8, 128), 0) < 4

        def w2_part(i):
            o_, n_ = w2_chunks[i]
            d = jnp.dot(lhs2[i], w2b[o_:o_ + n_, :], preferred_element_type=F32)
            return jnp.concatenate(
                [jnp.where(low, d[:, (2 * u) * 128:(2 * u + 1) * 128], d[:, (2 * u + 1) * 128:(2 * u + 2) * 128])
                 for u in range(2)], axis=0)

        for i in range(NM):
            w2_cps[i].wait()
            out = out + w2_part(i)
        acc = [[None] * 4 for _ in range(B)]
        for i in range(NM, len(w2_chunks)):
            o_, n_ = w2_chunks[i]
            w2_cps[i].wait()
            wf = w2b[o_:o_ + n_, :].astype(F32)
            for g in range(n_ // 8):
                for b in range(B):
                    pg = p_scr[b, o_ - (F - NV) + 8 * g:o_ - (F - NV) + 8 * g + 8, :]
                    for c in range(4):
                        t_ = pg * wf[8 * g:8 * g + 8, 128 * c:128 * (c + 1)]
                        acc[b][c] = t_ if acc[b][c] is None else acc[b][c] + t_
        sub = lax.broadcasted_iota(jnp.int32, (8, 128), 0)
        m4, m2, m1 = sub < 4, (sub % 4) < 2, (sub % 2) == 0

        def comb4(a_, b_):
            return jnp.where(m4, a_, b_) + pltpu.roll(jnp.where(m4, b_, a_), 4, 0)

        def comb(a_, b_, m_, sh):
            return jnp.where(m_, a_, b_) + jnp.where(m_, pltpu.roll(a_, 8 - sh, 0), pltpu.roll(b_, sh, 0))

        halves = []
        for u in range(2):
            l1 = [comb4(acc[b][2 * u], acc[b][2 * u + 1]) for b in range(B)]
            l2 = [comb(l1[0], l1[2], m2, 2), comb(l1[1], l1[3], m2, 2)]
            halves.append(comb(l2[0], l2[1], m1, 1))
        return out, jnp.concatenate(halves, axis=0)

    out, last = pl.run_scoped(
        stream_and_compute, *([pltpu.SemaphoreType.DMA(())] * (2 + len(W2_ROWS) + len(W2V_ROWS))))
    o_ref[...] = (out + last).astype(BF16)


@jax.jit
def pallas_gated_mix__gqa_block_cached__dense_activation_squared_relu__decode_kernel(
    A_x: jax.Array,
    A_k_cache: jax.Array,
    A_v_cache: jax.Array,
    A_wq: jax.Array,
    A_wo: jax.Array,
    B_x: jax.Array,
    B_w1: jax.Array,
    B_b1: jax.Array,
    B_w2: jax.Array,
    B_b2: jax.Array,
    gate_w: jax.Array,
):
    del B_x
    out = pl.pallas_call(
        _kernel,
        out_shape=jax.ShapeDtypeStruct((16, 128), BF16),
        in_specs=[pl.BlockSpec(memory_space=pl.ANY)] * 10,
        out_specs=pl.BlockSpec(memory_space=pltpu.VMEM),
        scratch_shapes=[
            pltpu.VMEM((B, D), BF16),
            pltpu.VMEM((NP, SK, DH), BF16),
            pltpu.VMEM((NP, SK, DH), BF16),
            pltpu.VMEM((D, HQ * DH), BF16),
            pltpu.VMEM((HQ * DH, D), BF16),
            pltpu.VMEM((D, F), BF16),
            pltpu.VMEM((F,), BF16),
            pltpu.VMEM((F, D), BF16),
            pltpu.VMEM((D,), BF16),
            pltpu.VMEM((D,), BF16),
            pltpu.VMEM((HKV, 16, DH), F32),
            pltpu.VMEM((HKV, 16, DH), F32),
            pltpu.VMEM((B, NV, 128), F32),
        ],
        compiler_params=pltpu.CompilerParams(vmem_limit_bytes=110 * 1024 * 1024),
    )(A_x.reshape(B, D), A_k_cache, A_v_cache, A_wq, A_wo, B_w1, B_b1, B_w2, B_b2, gate_w)
    return out.reshape(D // 128, B, 128).transpose(1, 0, 2).reshape(B, 1, D)
```
